```python
import os as _os
_os.environ.setdefault("JAX_PLATFORMS", "cpu")
import jax
import jax.numpy as jnp

def _softmax(x, axis=-1):
    return jax.nn.softmax(x, axis=axis)
def _gelu(x):
    return jax.nn.gelu(x, approximate=True)
def _silu(x):
    return jax.nn.silu(x)
def _sigmoid(x):
    return jax.nn.sigmoid(x)
def _layernorm(x, axis=-1, eps=1e-5):
    m = jnp.mean(x, axis=axis, keepdims=True)
    v = jnp.var(x, axis=axis, keepdims=True)
    return (x - m) / jnp.sqrt(v + eps)
def _scatter_add(tgt, idx, src, axis=0):
    return tgt.at[idx].add(src)
def _segment_sum(src, seg, n):
    return jax.ops.segment_sum(src, seg, n)
class _Rng:
    def __init__(self, key):
        self._k = key
    def _next(self):
        self._k, sub = jax.random.split(self._k)
        return sub
    def normal(self, shape):
        return jax.random.normal(self._next(), shape, dtype=jnp.bfloat16)
    def randint(self, lo, hi, shape):
        return jax.random.randint(self._next(), shape, lo, hi, dtype=jnp.int32)
    def uniform(self, shape, lo=0.0, hi=1.0):
        return jax.random.uniform(self._next(), shape, jnp.bfloat16, lo, hi)
    def permutation(self, n):
        return jax.random.permutation(self._next(), n)


kernel_name = 'sequential_preLN__sliding_block__glu_gated_swiglu__prompt'

def setup_inputs():
    _rng = _Rng(jax.random.key(int.from_bytes(__import__("os").urandom(4), "little")))
    _w = (lambda a: (lambda t: t.astype(jnp.bfloat16) if jnp.issubdtype(t.dtype, jnp.floating) else t)(jnp.asarray(a)))
    def _A_setup():
        B, S, D = 1, 2048, 640
        return {
            "x": _w((lambda *s: _rng.normal(s) * 0.05)(B, S, D)),
            "wqkv": _w((lambda *s: _rng.normal(s) * 0.05)(D, 3 * D)),
            "wo": _w((lambda *s: _rng.normal(s) * 0.05)(D, D)),
        }
    _A_in = _A_setup()

    def _B_setup():
        B, S, D, F = 1, 2048, 640, 1728
        return {
            "x": _w((lambda *s: _rng.normal(s) * 0.05)(B, S, D)),
            "w1": _w((lambda *s: _rng.normal(s) * 0.1)(D, F) * (2.0 / D) ** 0.5),
            "w3": _w((lambda *s: _rng.normal(s) * 0.1)(D, F) * (2.0 / D) ** 0.5),
            "w2": _w((lambda *s: _rng.normal(s) * 0.1)(F, D) * (2.0 / F) ** 0.5),
        }
    _B_in = _B_setup()

    return {
        "A_x": _A_in["x"],
        "A_wqkv": _A_in["wqkv"],
        "A_wo": _A_in["wo"],
        "B_x": _B_in["x"],
        "B_w1": _B_in["w1"],
        "B_w3": _B_in["w3"],
        "B_w2": _B_in["w2"],
    }

def reference(A_x, A_wqkv, A_wo, B_x, B_w1, B_w3, B_w2):
    def _A_ref(x, wqkv, wo):
        B, S, D = x.shape
        H = 32; Dh = D // H; W = 256
        qkv = (lambda x, *d: x.transpose(*d))((x @ wqkv).reshape(B, S, 3, H, Dh), 2, 0, 3, 1, 4)
        q, k, v = qkv[0], qkv[1], qkv[2]
        scores = jnp.einsum("bhqd,bhkd->bhqk", q, k) * (Dh ** -0.5)
        idx = jnp.arange(S)
        mask = (idx[:, None] - idx[None, :] >= 0) & (idx[:, None] - idx[None, :] < W)
        scores = jnp.where(mask[None, None], scores, -1e9)
        p = _softmax(scores, axis=-1)
        o = jnp.einsum("bhqk,bhkd->bhqd", p, v)
        return (lambda x, *d: x.transpose(*d))(o, 0, 2, 1, 3).reshape(B, S, D) @ wo

    def _B_ref(x, w1, w3, w2):
        gate = jnp.einsum("bsd,df->bsf", x, w1)
        up = jnp.einsum("bsd,df->bsf", x, w3)
        h = _silu(gate) * up
        out = jnp.einsum("bsf,fd->bsd", h, w2)
        return out

    x = A_x
    h = x + _A_ref(_layernorm(x, axis=-1), A_wqkv, A_wo)
    h2 = h + _B_ref(_layernorm(h, axis=-1), B_w1, B_w3, B_w2)
    return h2
```

```python
import functools
import math

import jax
import jax.numpy as jnp
import jax.experimental.pallas as pl
import jax.experimental.pallas.tpu as pltpu

S, D, H, DH, WIN, F = 2048, 640, 32, 20, 256, 1728
T = 256
NSTEP = S // T
NW = 6
EPS = 1e-5
QSCALE = (DH ** -0.5) * math.log2(math.e)
NEG = -1e30
LAG = 2
GRP = 1
f32 = jnp.float32
bf16 = jnp.bfloat16


def _ln(x):
    m = jnp.mean(x, axis=-1, keepdims=True)
    xc = x - m
    v = jnp.mean(xc * xc, axis=-1, keepdims=True)
    return xc * jax.lax.rsqrt(v + EPS)


def _windows(a):
    lane = jax.lax.broadcasted_iota(jnp.int32, (a.shape[0], 128), 1)
    tiles = [a[:, 128 * t:128 * (t + 1)] for t in range(5)]
    out = [tiles[0]]
    for w in range(1, 5):
        out.append(jnp.where(lane < 128 - 8 * w, tiles[w], tiles[w - 1]))
    out.append(tiles[4])
    return out


def _nt(a, b):
    return jax.lax.dot_general(a, b, (((1,), (1,)), ((), ())), preferred_element_type=f32)


def _body(first, step, x_ref, o_ref, wqkv, wo, w1t, w3t, w2, wvt, k_s, vt_s, waits):
    cur = step + 1
    prev = step
    x = x_ref[...].astype(f32)
    xn = _ln(x).astype(bf16)
    waits[0]()
    if first:
        wvt[...] = wqkv[:, 2 * D:3 * D].astype(f32).T.astype(bf16)
    qk = jnp.dot(xn, wqkv[:, :2 * D], preferred_element_type=f32)
    qw = _windows(qk[:, :D] * QSCALE)
    kw = _windows(qk[:, D:])
    for w in range(NW):
        k_s[cur, :, 128 * w:128 * (w + 1)] = kw[w].astype(bf16)
    vt = _nt(wvt[...], xn)
    sub8t = jax.lax.broadcasted_iota(jnp.int32, (8, T), 0)
    ones16 = jnp.ones((16, T), f32)
    ev, od = [], []
    for p in range(H // 2):
        mid = vt[40 * p + 16:40 * p + 24]
        ev += [vt[40 * p:40 * p + 16], jnp.where(sub8t < 4, mid, 1.0), ones16]
        od += [ones16, jnp.where(sub8t < 4, 1.0, mid), vt[40 * p + 24:40 * p + 40]]
    vt_s[cur, 0] = jnp.concatenate(ev, axis=0).astype(bf16)
    vt_s[cur, 1] = jnp.concatenate(od, axis=0).astype(bf16)

    lane64 = jax.lax.broadcasted_iota(jnp.int32, (64, 128), 1)
    row64 = jax.lax.broadcasted_iota(jnp.int32, (64, 128), 0)
    tri = row64 > (lane64 % 64)
    sub8 = jax.lax.broadcasted_iota(jnp.int32, (8, 128), 0)

    def scores(b, p):
        w = p // 3 if p < 15 else 5
        out = []
        for j in range(2):
            q0 = 128 * b + 64 * j
            qsub = qw[w][q0:q0 + 64]
            parts = [None, None]
            for h in range(2):
                lo = (40 * p + 20 * h) % 128
                hi = lo + 20
                if hi <= 128:
                    msk = (lane64 >= lo) & (lane64 < hi)
                else:
                    msk = (lane64 >= lo) | (lane64 < hi - 128)
                parts[(h + j) % 2] = jnp.where(msk, qsub, 0.0)
            wt = jnp.concatenate(parts, axis=0).astype(bf16)
            kc = k_s[cur, 0:q0 + 64, 128 * w:128 * (w + 1)]
            if not first:
                kp = k_s[prev, q0:T, 128 * w:128 * (w + 1)]
                kc = jnp.concatenate([kp, kc], axis=0)
            out.append(_nt(kc, wt))
        return out

    def softpv(b, p, ss):
        pj = []
        z = jnp.zeros((64, 128), f32)
        for j in range(2):
            q0 = 128 * b + 64 * j
            s = ss[j]
            if first:
                bot = jnp.where(tri, NEG, s[q0:])
                sm = bot if q0 == 0 else jnp.concatenate([s[:q0], bot], axis=0)
                m = jnp.max(sm, axis=0, keepdims=True)
                pu = jnp.exp2(sm - m)
                if j == 0:
                    pu = jnp.concatenate([pu, z], axis=0)
            else:
                mer = jnp.where(tri, s[:64], s[256:])
                sm = jnp.concatenate([mer, s[64:256]], axis=0)
                m = jnp.max(sm, axis=0, keepdims=True)
                pm = jnp.exp2(sm - m)
                lst = [jnp.where(tri, pm[:64], 0.0), pm[64:], jnp.where(tri, 0.0, pm[:64])]
                pu = jnp.concatenate(lst + [z] if j == 0 else [z] + lst, axis=0)
            pj.append(pu)
        lanek = jax.lax.broadcasted_iota(jnp.int32, pj[0].shape, 1)
        res = []
        for h in range(2):
            hh = 2 * p + h
            ph = jnp.where(lanek < 64, pj[h], pj[1 - h]).astype(bf16)
            r0 = 80 * (hh // 4) + 16 * (hh % 4)
            vc = vt_s[cur, h, r0:r0 + 32, 0:128 * (b + 1)]
            if not first:
                vp = vt_s[prev, h, r0:r0 + 32, 128 * b:T]
                vc = jnp.concatenate([vp, vc], axis=1)
            r = jnp.dot(vc, ph, preferred_element_type=f32)
            if hh % 4 < 2:
                l, o = r[24:32], r[0:24]
            else:
                l, o = r[0:8], r[8:32]
            inv = 1.0 / l
            o = o * jnp.concatenate([inv, inv, inv], axis=0)
            if h == 1:
                o = pltpu.roll(o, 64, 1)
            res.append(o)
        a, c = res
        return jnp.concatenate([a[0:16], jnp.where(sub8 < 4, a[16:24], c[0:8]), c[8:24]], axis=0)

    units = [(b, p) for b in range(T // 128) for p in range(H // 2)]
    groups = [units[i:i + GRP] for i in range(0, len(units), GRP)]
    sc, res = {}, {}
    for gi in range(len(groups) + LAG):
        if gi < len(groups):
            for u in groups[gi]:
                sc[u] = scores(*u)
        if gi >= LAG:
            for u in groups[gi - LAG]:
                res[u] = softpv(*u, sc.pop(u))
    ot = jnp.concatenate(
        [jnp.concatenate([res[(b, p)] for p in range(H // 2)], axis=0) for b in range(T // 128)], axis=1)
    o = ot.T.astype(bf16)
    waits[1]()
    h1 = x + jnp.dot(o, wo[...], preferred_element_type=f32)
    hn = _ln(h1).astype(bf16)
    waits[2]()
    acts = []
    for c in range(14):
        n = 128 if c < 13 else 64
        wt = jnp.concatenate([w1t[128 * c:128 * c + n], w3t[128 * c:128 * c + n]], axis=0)
        gu = _nt(hn, wt)
        if c < 13:
            g, u = gu[:, :128], gu[:, 128:]
        else:
            g, u = gu, pltpu.roll(gu, 64, 1)
        hg = 0.5 * g
        a = (hg * jnp.tanh(hg) + hg) * u
        acts.append(a if c < 13 else a[:, :64])
    a = jnp.concatenate(acts, axis=1).astype(bf16)
    waits[3]()
    o_ref[...] = (h1 + jnp.dot(a, w2[...], preferred_element_type=f32)).astype(o_ref.dtype)


def _kernel(x_ref, wqkv_h, wo_h, w1_h, w3_h, w2_h, o_ref,
            wqkv, wo, w1, w3, w2, wvt, k_s, vt_s, sems):
    step = pl.program_id(0)
    args = (x_ref, o_ref, wqkv, wo, w1, w3, w2, wvt, k_s, vt_s)

    @pl.when(step == 0)
    def _():
        cps = [pltpu.make_async_copy(s, d, sems.at[i]) for i, (s, d) in enumerate(
            [(wqkv_h, wqkv), (wo_h, wo), (w1_h, w1), (w3_h, w3), (w2_h, w2)])]
        for c in cps:
            c.start()

        def w13():
            cps[2].wait()
            cps[3].wait()
        _body(True, step, *args, [cps[0].wait, cps[1].wait, w13, cps[4].wait])

    @pl.when(step > 0)
    def _():
        nop = lambda: None
        _body(False, step, *args, [nop] * 4)


@jax.jit
def pallas_sequential_preLN__sliding_block__glu_gated_swiglu__prompt_kernel(A_x, A_wqkv, A_wo, B_x, B_w1, B_w3, B_w2):
    x = A_x.reshape(S, D)
    anyspec = pl.BlockSpec(memory_space=pltpu.HBM)
    out = pl.pallas_call(
        _kernel,
        grid=(NSTEP,),
        in_specs=[pl.BlockSpec((T, D), lambda i: (i, 0))] + [anyspec] * 5,
        out_specs=pl.BlockSpec((T, D), lambda i: (i, 0)),
        out_shape=jax.ShapeDtypeStruct((S, D), bf16),
        scratch_shapes=[
            pltpu.VMEM((D, 3 * D), bf16), pltpu.VMEM((D, D), bf16),
            pltpu.VMEM((F, D), bf16), pltpu.VMEM((F, D), bf16), pltpu.VMEM((F, D), bf16),
            pltpu.VMEM((D, D), bf16),
            pltpu.VMEM((NSTEP + 1, T, NW * 128), bf16),
            pltpu.VMEM((NSTEP + 1, 2, D, T), bf16),
            pltpu.SemaphoreType.DMA((5,)),
        ],
        compiler_params=pltpu.CompilerParams(
            dimension_semantics=("arbitrary",), vmem_limit_bytes=100 * 1024 * 1024),
        name="fused_block",
    )(x, A_wqkv, A_wo, B_w1.T, B_w3.T, B_w2)
    return out.reshape(1, S, D)
```

```python
import math

import jax
import jax.numpy as jnp
import jax.experimental.pallas as pl
import jax.experimental.pallas.tpu as pltpu

S, D, H, DH, WIN, F = 2048, 640, 32, 20, 256, 1728
T = 256
NB = S // T
NW = 8
EPS = 1e-5
QSCALE = (DH ** -0.5) * math.log2(math.e)
NEG = -1e30
LAG = 1
LAGP = 2
NRING = 16
CPRE = 18
CMID = 335
SLOTS = [18] * 12 + [10, 28, 21, 28, 0]
ORD0 = 1
ORD1 = 0
AHEAD = 2
TAIL = 2
OEARLY = 1
SUP = (0, 3, 4, 6, 2, 1, 5)
SUP_S = (0, 3, 4, 6, 2, 1, 5)
SDN = (0, 3, 4, 6, 2, 1, 5)
SDN_S = (4, 2, 1, 3, 0, 6, 5)
CHECKS = False
SORD = (0, 3, 4, 6, 2, 1, 5)
f32 = jnp.float32
bf16 = jnp.bfloat16
RIDX = {0: 0, 2: 1, 3: 2, 5: 3, 6: 4}
LIDX = {0: 0, 1: 1, 4: 2, 5: 3, 6: 4}


def _ln(x):
    m = jnp.mean(x, axis=-1, keepdims=True)
    xc = x - m
    v = jnp.mean(xc * xc, axis=-1, keepdims=True)
    return xc * jax.lax.rsqrt(v + EPS)


def _window(tiles, g):
    t0, t1 = (80 * g) // 128, (80 * g + 79) // 128
    if t0 == t1:
        return tiles[t0]
    lane = jax.lax.broadcasted_iota(jnp.int32, tiles[t0].shape, 1)
    return jnp.where(lane >= (80 * g) % 128, tiles[t0], tiles[t1])


def _nn(a, b):
    return jnp.dot(a, b, preferred_element_type=f32)


def _nt(a, b):
    return jax.lax.dot_general(a, b, (((1,), (1,)), ((), ())), preferred_element_type=f32)


def _lhs7(a11, a12, a21, a22):
    return [a11 + a22, a21 + a22, a11, a22, a11 + a12, a21 - a11, a12 - a22]


def _lhs7_of(a):
    h = a.shape[0] // 2
    return _lhs7(a[:h, 0:256], a[:h, 256:512], a[h:, 0:256], a[h:, 256:512])


def _rhs(fly, cache, b11, b12, b21, b22):
    terms = {0: (b11, b22, 1), 2: (b12, b22, -1), 3: (b21, b11, -1), 5: (b11, b12, 1), 6: (b21, b22, 1)}

    def get(i):
        if i == 1:
            return b11()
        if i == 4:
            return b22()
        ref = cache(RIDX[i])
        if not fly:
            return ref[...]
        p, q, sgn = terms[i]
        p, q = p().astype(f32), q().astype(f32)
        s = p + q if sgn > 0 else p - q
        h = s.shape[0] // 2
        ref[0:h] = s[:h].astype(bf16)
        ref[h:2 * h] = s[h:].astype(bf16)
        return s.astype(bf16)
    return get


def _products_gen(mm, lhs, rhs, cost, order=None):
    m = [None] * 7
    for i in (order or SORD):
        m[i] = mm(lhs(i), rhs(i))
        yield cost
    return (m[0] + m[3] - m[4] + m[6], m[2] + m[4], m[1] + m[3], m[0] - m[1] + m[2] + m[5])


def _products(mm, lhs, rhs):
    gen = _products_gen(mm, lhs, rhs, 0)
    while True:
        try:
            next(gen)
        except StopIteration as e:
            return e.value


class _Fill:
    def __init__(self, gen):
        self.gen, self.done = gen, 0

    def advance(self, target=1e9):
        while self.done < target - 1e-6:
            try:
                self.done += next(self.gen)
            except StopIteration:
                return


def _w2rows(w2, par, cs):
    rows = [w2[256 * k + 128 * par:256 * k + 128 * par + 128, cs] for k in range(7 - par)]
    if par:
        rows += [w2[1664:1728, cs], jnp.zeros((64, cs.stop - cs.start), bf16)]
    return rows


def _ffn(r, blk, solo):
    fly = solo
    acts = []
    ll = [[] for _ in range(7)]

    def hop(i):
        if i == 2:
            return r.hn[blk, 0:128, 0:256]
        if i == 3:
            return r.hn[blk, 128:256, 256:512]
        return r.hs[blk, LIDX[i]]

    for c in range(14):
        if c < 13:
            rs = slice(128 * c, 128 * c + 128)
            rhs = _rhs(fly, lambda s: r.wup.at[s, rs],
                       lambda: r.w1[rs, 0:256], lambda: r.w3[rs, 0:256],
                       lambda: r.w1[rs, 256:512], lambda: r.w3[rs, 256:512])
            rem = _nt(r.hn[blk, :, 512:640],
                      jnp.concatenate([r.w1[rs, 512:640], r.w3[rs, 512:640]], axis=0))
            yield 4
            c11, c12, c21, c22 = yield from _products_gen(_nt, hop, rhs, 2, SUP_S if solo else SUP)
            g = jnp.concatenate([c11, c21], axis=0) + rem[:, :128]
            u = jnp.concatenate([c12, c22], axis=0) + rem[:, 128:]
        else:
            wt = jnp.concatenate([r.w1[1664:1728], r.w3[1664:1728]], axis=0)
            g = _nt(r.hn[blk], wt)
            yield 10
            u = pltpu.roll(g, 64, 1)
        hg = 0.5 * g
        a = (hg * jnp.tanh(hg) + hg) * u
        if c == 13:
            lane = jax.lax.broadcasted_iota(jnp.int32, a.shape, 1)
            a = jnp.where(lane < 64, a, 0.0)
        acts.append(a)
        if c % 2 == 1:
            e, o = acts[c - 1], acts[c]
            for lst, v in zip(ll, _lhs7(e[:128], o[:128], e[128:], o[128:])):
                lst.append(v)

    def finish(cs, y):
        r.o[blk, :, cs] = (r.h1[blk, :, cs] + y).astype(bf16)
        if solo:
            pltpu.make_async_copy(r.o.at[blk, :, cs], r.oh.at[blk, :, cs], r.osem).start()

    lb = [jnp.concatenate(lst, axis=1).astype(bf16) for lst in ll]

    def down2(n0, n1):
        c0, c1 = slice(128 * n0, 128 * n1), slice(256 + 128 * n0, 256 + 128 * n1)

        def blk2(par, cs):
            return lambda: jnp.concatenate([v.astype(f32) for v in _w2rows(r.w2, par, cs)], axis=0)
        rhs = _rhs(fly, lambda s: r.wdn.at[s, :, c0], blk2(0, c0), blk2(0, c1), blk2(1, c0), blk2(1, c1))

        def rhs2(i):
            if i == 1:
                return jnp.concatenate(_w2rows(r.w2, 0, c0), axis=0)
            if i == 4:
                return jnp.concatenate(_w2rows(r.w2, 1, c1), axis=0)
            return rhs(i)
        c11, c12, c21, c22 = yield from _products_gen(_nn, lambda i: lb[i], rhs2, 7 * (n1 - n0), SDN_S if solo else SDN)
        finish(c0, jnp.concatenate([c11, c21], axis=0))
        finish(c1, jnp.concatenate([c12, c22], axis=0))

    def down1():
        a = jnp.concatenate(acts[:13] + [acts[13][:, :64]], axis=1).astype(bf16)
        cs = slice(512, 640)
        finish(cs, _nn(a, r.w2[:, cs]))
        yield 28

    if solo:
        yield from down2(0, 2)
        yield from down1()
    else:
        yield from down2(0, 1)
        yield from down1()
        yield from down2(1, 2)
        pltpu.make_async_copy(r.o.at[blk], r.oh.at[blk], r.osem).start()


class _Proj:
    def __init__(self, r, blk, qs):
        self.r, self.blk, self.qs = r, blk, qs
        self._xf = self._xn = self._l7 = None
        self.kt, self.qt = [], []

    def xf(self):
        if self._xf is None:
            self._xf = _ln(self.r.x[self.blk].astype(f32))
        return self._xf

    def xn(self):
        if self._xn is None:
            self._xn = self.xf().astype(bf16)
        return self._xn

    def l7(self):
        if self._l7 is None:
            self._l7 = [v.astype(bf16) for v in _lhs7_of(self.xf())] + [self.xf()[:, 512:640].astype(bf16)]
        return self._l7

    def put(self, y):
        isq = len(self.qt) < 5
        tiles = self.qt if isq else self.kt
        tiles.append(y)
        for g in range(NW):
            if (80 * g + 79) // 128 == len(tiles) - 1:
                if isq:
                    self.r.q[self.qs, g] = _window(tiles, g) * QSCALE
                else:
                    self.r.k[self.blk + 1, :, 128 * g:128 * (g + 1)] = _window(tiles, g).astype(bf16)

    def put_v(self, vt, p0):
        r = self.r
        sub8t = jax.lax.broadcasted_iota(jnp.int32, (8, T), 0)
        ones16 = jnp.ones((16, T), f32)
        ev, od = [], []
        n = vt.shape[0] // 40
        for p in range(n):
            mid = vt[40 * p + 16:40 * p + 24]
            ev += [vt[40 * p:40 * p + 16], jnp.where(sub8t < 4, mid, 1.0), ones16]
            od += [ones16, jnp.where(sub8t < 4, 1.0, mid), vt[40 * p + 24:40 * p + 40]]
        r.vt[self.blk + 1, 0, 40 * p0:40 * (p0 + n)] = jnp.concatenate(ev, axis=0).astype(bf16)
        r.vt[self.blk + 1, 1, 40 * p0:40 * (p0 + n)] = jnp.concatenate(od, axis=0).astype(bf16)

    def qk(self, p0, p1, fly=False):
        r, l7 = self.r, self.l7()
        for p in range(p0, p1):
            ca, cb = slice(256 * p, 256 * p + 128), slice(256 * p + 128, 256 * p + 256)
            rhs = _rhs(fly, lambda s: r.wqk.at[s, :, 128 * p:128 * p + 128],
                       lambda: r.wqkv[0:256, ca], lambda: r.wqkv[0:256, cb],
                       lambda: r.wqkv[256:512, ca], lambda: r.wqkv[256:512, cb])
            rem = _nn(l7[7], r.wqkv[512:640, 256 * p:256 * p + 256])
            c11, c12, c21, c22 = _products(_nn, lambda i: l7[i], rhs)
            self.put(jnp.concatenate([c11, c21], axis=0) + rem[:, :128])
            self.put(jnp.concatenate([c12, c22], axis=0) + rem[:, 128:])

    def v(self, fly=False):
        r, l7 = self.r, self.l7()
        rhs = _rhs(fly, lambda s: r.wvs.at[s],
                   lambda: r.wvt[0:320, 0:256], lambda: r.wvt[320:640, 0:256],
                   lambda: r.wvt[0:320, 256:512], lambda: r.wvt[320:640, 256:512])
        rem = _nt(r.wvt[:, 512:640], l7[7])
        c11, c12, c21, c22 = _products(lambda a, b: _nt(b, a), lambda i: l7[i], rhs)
        vt = jnp.concatenate([jnp.concatenate([c11, c21], axis=1),
                              jnp.concatenate([c12, c22], axis=1)], axis=0) + rem
        self.put_v(vt, 0)


class _Attn:
    def __init__(self, r, blk, first, qs):
        self.r, self.blk, self.first, self.qs = r, blk, first, qs
        self.sc, self.res = {}, {}
        self.units = [(self, b, g) for b in range(T // 128) for g in range(NW)]

    def scores(self, b, g):
        r, first = self.r, self.first
        cur, prev = self.blk + 1, self.blk
        lane32 = jax.lax.broadcasted_iota(jnp.int32, (32, 128), 1)
        row32 = jax.lax.broadcasted_iota(jnp.int32, (32, 128), 0)
        tri = row32 > (lane32 % 32)
        cs = slice(128 * g, 128 * (g + 1))
        ns = []
        for j in range(4):
            q0 = 128 * b + 32 * j
            qsub = r.q[self.qs, g, q0:q0 + 32]
            parts = [None] * 4
            for h in range(4):
                lo = (80 * g + 20 * h) % 128
                hi = lo + 20
                if hi <= 128:
                    msk = (lane32 >= lo) & (lane32 < hi)
                else:
                    msk = (lane32 >= lo) | (lane32 < hi - 128)
                parts[(h + j) % 4] = jnp.where(msk, qsub, 0.0)
            wt = jnp.concatenate(parts, axis=0).astype(bf16)
            if first:
                s = _nt(r.k[cur, 0:q0 + 32, cs], wt)
                lst = ([s[:q0]] if q0 else []) + [jnp.where(tri, NEG, s[q0:])]
                if j < 3:
                    lst.append(jnp.full((96 - 32 * j, 128), NEG, f32))
                ns.append(jnp.concatenate(lst, axis=0))
            else:
                def krows(r0, r1):
                    a0, a1 = q0 + r0, q0 + r1
                    if a0 == a1:
                        return []
                    if a1 <= T:
                        return [r.k[prev, a0:a1, cs]]
                    if a0 >= T:
                        return [r.k[cur, a0 - T:a1 - T, cs]]
                    return [r.k[prev, a0:T, cs], r.k[cur, 0:a1 - T, cs]]
                o = 32 * j
                kc = (krows(256 - o, 256) + krows(0, 16) + krows(256, 272) + krows(16, 32)
                      + krows(272, 288) + krows(32, 256 - o))
                s = _nt(jnp.concatenate(kc, axis=0), wt)
                top = jnp.concatenate([s[o:o + 16], s[o + 32:o + 48]], axis=0)
                bot = jnp.concatenate([s[o + 16:o + 32], s[o + 48:o + 64]], axis=0)
                mer = jnp.where(tri, top, bot)
                ns.append(jnp.concatenate(([s[:o]] if j else []) + [mer, s[o + 64:]], axis=0))
        lane = jax.lax.broadcasted_iota(jnp.int32, ns[0].shape, 1)
        odd = (lane % 64) >= 32
        aa = [jnp.where(odd, ns[(j + 1) % 4], ns[j]) for j in range(4)]
        out = []
        for h in range(4):
            j = (4 - h) % 4
            sm = jnp.where(lane >= 64, aa[(j + 2) % 4], aa[j])
            sl = r.ring[0]
            r.ring[0] = (sl + 1) % NRING
            n = sm.shape[0]
            r.s[sl, 0:n] = sm
            out.append((sl, n, jnp.max(sm, axis=0, keepdims=True)))
        self.sc[(b, g)] = out

    def softpv(self, b, g):
        r, first = self.r, self.first
        cur, prev = self.blk + 1, self.blk
        sub8 = jax.lax.broadcasted_iota(jnp.int32, (8, 128), 0)
        lane128 = jax.lax.broadcasted_iota(jnp.int32, (128, 128), 1)
        row128 = jax.lax.broadcasted_iota(jnp.int32, (128, 128), 0)
        ss = self.sc.pop((b, g))
        res = []
        for h in range(4):
            sl, n, m = ss[h]
            pm = jnp.exp2(r.s[sl, 0:n] - m)
            if not first:
                trih = row128 > ((lane128 + 128 - 32 * h) % 128)
                pm = jnp.concatenate([jnp.where(trih, pm[:128], 0.0), pm[128:],
                                      jnp.where(trih, 0.0, pm[:128])], axis=0)
            ph = pm.astype(bf16)
            r0 = 80 * g + 16 * h
            vc = r.vt[cur, h % 2, r0:r0 + 32, 0:128 * (b + 1)]
            if not first:
                vp = r.vt[prev, h % 2, r0:r0 + 32, 128 * b:T]
                vc = jnp.concatenate([vp, vc], axis=1)
            y = _nn(vc, ph)
            if h < 2:
                l, o = y[24:32], y[0:24]
            else:
                l, o = y[0:8], y[8:32]
            inv = 1.0 / l
            o = o * jnp.concatenate([inv, inv, inv], axis=0)
            if h:
                o = pltpu.roll(o, 128 - 32 * h, 1)
            res.append(o)
        rows = []
        for a, c in (res[0:2], res[2:4]):
            rows += [a[0:16], jnp.where(sub8 < 4, a[16:24], c[0:8]), c[8:24]]
        self.res[(b, g)] = jnp.concatenate(rows, axis=0)

    def oproj(self, fly=False):
        r = self.r
        o = jnp.concatenate(
            [jnp.concatenate([self.res[(b, g)] for g in range(NW)], axis=0)
             for b in range(T // 128)], axis=1).T
        l7 = [v.astype(bf16) for v in _lhs7_of(o)]
        rhs = _rhs(fly, lambda s: r.wos.at[s],
                   lambda: r.wo[0:256, 0:256], lambda: r.wo[0:256, 256:512],
                   lambda: r.wo[256:512, 0:256], lambda: r.wo[256:512, 256:512])
        c11, c12, c21, c22 = _products(_nn, lambda i: l7[i], rhs)
        y = jnp.concatenate([jnp.concatenate([c11, c12], axis=1),
                             jnp.concatenate([c21, c22], axis=1)], axis=0)
        y = y + _nn(o[:, 512:640].astype(bf16), r.wo[512:640, 0:512])
        y = jnp.concatenate([y, _nn(o.astype(bf16), r.wo[:, 512:640])], axis=1)
        h1 = r.x[self.blk].astype(f32) + y
        r.h1[self.blk] = h1
        hn = _ln(r.h1[self.blk])
        r.hn[self.blk] = hn.astype(bf16)
        ops = _lhs7_of(hn)
        for i, sl in LIDX.items():
            r.hs[self.blk, sl] = ops[i].astype(bf16)


def _pipeline(units, lag, between):
    for i in range(len(units) + lag):
        if i < len(units):
            a, b, g = units[i]
            a.scores(b, g)
        between(i)
        if i >= lag:
            a, b, g = units[i - lag]
            a.softpv(b, g)


def _steady(r, blk):
    fill = _Fill(_ffn(r, blk - 1, False))
    fill.advance(CPRE)
    p = _Proj(r, blk, 0)
    p.qk(0, 5)
    p.v()
    at = _Attn(r, blk, False, 0)
    nslot = len(at.units) + LAG
    _pipeline(at.units, LAG,
              lambda i: fill.advance(CPRE + sum(SLOTS[:i + 1])))
    fill.advance(CMID)
    at.oproj()
    fill.advance()


class _Refs:
    pass


def _kernel(x_h, wqkv_h, wo_h, w1_h, w3_h, w2_h, o_h,
            x_s, o_s, wqkv, wo, w1, w3, w2, wvt, wqk, wvs, wos, wup, wdn,
            k_s, vt_s, h1_s, hn_s, hs_s, s_s, q_s, sems, osem):
    r = _Refs()
    r.x, r.o, r.wqkv, r.wo, r.w1, r.w3, r.w2, r.wvt = x_s, o_s, wqkv, wo, w1, w3, w2, wvt
    r.wqk, r.wvs, r.wos, r.wup, r.wdn = wqk, wvs, wos, wup, wdn
    r.k, r.vt, r.h1, r.hn, r.hs = k_s, vt_s, h1_s, hn_s, hs_s
    r.s, r.ring, r.q = s_s, [0], q_s
    r.oh, r.osem = o_h, osem

    def xcopy(blk):
        return pltpu.make_async_copy(x_h.at[blk], x_s.at[blk], sems.at[8 + blk])

    def prologue():
        def wcol(c0, c1):
            return wqkv_h.at[:, c0:c1], wqkv.at[:, c0:c1]
        cx0, cx1 = xcopy(0), xcopy(1)
        pairs = [wcol(0, 256), wcol(256, 768), wcol(768, 2 * D), wcol(2 * D, 3 * D),
                 (wo_h, wo), (w1_h, w1), (w3_h, w3), (w2_h, w2)]
        cps = [pltpu.make_async_copy(s, d, sems.at[i]) for i, (s, d) in enumerate(pairs)]
        for c in [cx0, cx1] + cps:
            c.start()
        for blk in range(2, NB):
            xcopy(blk).start()
        ca, cb, cc, cv, cwo, cw1, cw3, cw2 = cps
        p0, p1 = _Proj(r, 0, 0), _Proj(r, 1, 1)
        cx0.wait()
        p0.l7()
        cx1.wait()
        p1.l7()
        ca.wait()
        p0.qk(0, 1, True)
        p1.qk(0, 1)
        cb.wait()
        p0.qk(1, 3, True)
        p1.qk(1, 3)
        cc.wait()
        p0.qk(3, 5, True)
        p1.qk(3, 5)
        cv.wait()
        cwo.wait()
        wvt[...] = wqkv[:, 2 * D:3 * D].astype(f32).T.astype(bf16)
        a0, a1 = _Attn(r, 0, True, 0), _Attn(r, 1, False, 1)
        big = list(a1.units) if ORD1 == 0 else sorted(a1.units, key=lambda u: (u[2], u[1]))
        small = sorted(a0.units, key=(lambda u: (u[2], -u[1])) if ORD0 else (lambda u: (u[1], u[2])))
        units = big[:AHEAD]
        big = big[AHEAD:]
        nb, ns = len(big) - TAIL, len(small)
        k = 0
        for i in range(nb):
            while k < ns and k * nb < (i + 1) * ns:
                units.append(small[k])
                k += 1
            units.append(big[i])
        units += big[nb:]

        def between(i):
            if i == LAGP:
                p0.v(True)
                p1.v()
            if i == len(units) + LAGP - OEARLY:
                a0.oproj(True)
        _pipeline(units, LAGP, between)
        a1.oproj()
        cw1.wait()
        cw3.wait()
        cw2.wait()

    def step(i, carry):
        pl.when(i == 0)(prologue)

        @pl.when((i > 1) & (i < NB))
        def _():
            xcopy(i).wait()
            _steady(r, i)

        @pl.when((i == 1) | (i == NB))
        def _():
            _Fill(_ffn(r, i - 1, True)).advance()
        return carry
    jax.lax.fori_loop(0, NB + 1, step, 0)
    pltpu.make_async_copy(o_s, o_h, osem).wait()


@jax.jit
def pallas_sequential_preLN__sliding_block__glu_gated_swiglu__prompt_kernel(A_x, A_wqkv, A_wo, B_x, B_w1, B_w3, B_w2):
    x = A_x.reshape(NB, T, D)
    hbm = pl.BlockSpec(memory_space=pltpu.HBM)
    out = pl.pallas_call(
        _kernel,
        in_specs=[hbm] * 6,
        out_specs=hbm,
        out_shape=jax.ShapeDtypeStruct((NB, T, D), bf16),
        scratch_shapes=[
            pltpu.VMEM((NB, T, D), bf16), pltpu.VMEM((NB, T, D), bf16),
            pltpu.VMEM((D, 3 * D), bf16), pltpu.VMEM((D, D), bf16),
            pltpu.VMEM((F, D), bf16), pltpu.VMEM((F, D), bf16), pltpu.VMEM((F, D), bf16),
            pltpu.VMEM((D, D), bf16),
            pltpu.VMEM((5, 256, D), bf16), pltpu.VMEM((5, 320, 256), bf16),
            pltpu.VMEM((5, 256, 256), bf16), pltpu.VMEM((5, 1664, 256), bf16),
            pltpu.VMEM((5, 896, 256), bf16),
            pltpu.VMEM((NB + 1, T, NW * 128), bf16),
            pltpu.VMEM((NB + 1, 2, D, T), bf16),
            pltpu.VMEM((NB, T, D), f32), pltpu.VMEM((NB, T, D), bf16),
            pltpu.VMEM((NB, 5, 128, 256), bf16),
            pltpu.VMEM((NRING, T, 128), f32), pltpu.VMEM((2, NW, T, 128), f32),
            pltpu.SemaphoreType.DMA((8 + NB,)), pltpu.SemaphoreType.DMA(()),
        ],
        compiler_params=pltpu.CompilerParams(vmem_limit_bytes=100 * 1024 * 1024,
                                             disable_bounds_checks=not CHECKS,
                                             disable_semaphore_checks=not CHECKS),
        name="fused_block",
    )(x, A_wqkv, A_wo, B_w1.T, B_w3.T, B_w2)
    return out.reshape(1, S, D)
```

```python
import math

import jax
import jax.numpy as jnp
import jax.experimental.pallas as pl
import jax.experimental.pallas.tpu as pltpu

S, D, DH, F = 2048, 640, 20, 1728
T = 256
NB = S // T
NW = 8
EPS = 1e-5
QSCALE = (DH ** -0.5) * math.log2(math.e)
NEG = -1e30
NRING = 16
NPART = 64
LAG = 1
LAGP = 2
SLOTS = [20, 22, 19] + [16] * 12 + [12, 12]
CMID = 289
SHIFT = 4
PIN = 12
f32 = jnp.float32
bf16 = jnp.bfloat16


def _ln_rows(x, dep):
    t = x[:, 0:128] if dep is None else x[:, 0:128] + dep
    for c in range(1, 5):
        t = t + x[:, 128 * c:128 * (c + 1)]
    m = jnp.sum(t, axis=-1, keepdims=True) * (1.0 / D)
    xc = x - m
    v = jnp.mean(xc * xc, axis=-1, keepdims=True)
    rs = jax.lax.rsqrt(v + EPS)
    return xc * rs, rs * 0.0


def _ln_pairs(load, rows):
    da = db = None
    for s in range(0, 128, rows):
        ra, rb = slice(s, s + rows), slice(128 + s, 128 + s + rows)
        a, da = _ln_rows(load(ra), da)
        b, db = _ln_rows(load(rb), db)
        yield ra, rb, a, b, da + db


def _window(tiles, g):
    t0, t1 = (80 * g) // 128, (80 * g + 79) // 128
    if t0 == t1:
        return tiles[t0]
    lane = jax.lax.broadcasted_iota(jnp.int32, tiles[t0].shape, 1)
    return jnp.where(lane >= (80 * g) % 128, tiles[t0], tiles[t1])


def _nn(a, b):
    return jnp.dot(a, b, preferred_element_type=f32)


def _nt(a, b):
    return jax.lax.dot_general(a, b, (((1,), (1,)), ((), ())), preferred_element_type=f32)


class _Fill:
    def __init__(self, gen):
        self.gen, self.done = gen, 0

    def advance(self, target=10 ** 9):
        while self.done < target:
            try:
                self.done += next(self.gen)
            except StopIteration:
                return


def _hk_plan(diags, pairs):
    def diff(i, k2, k):
        return (("d", i, k2, k), 1) if k2 > k else (("d", i, k, k2), -1)
    ext = {c: ([], []) for c in diags}
    pp = {}
    for c, c2 in pairs:
        (k, n), (k2, n2) = c, c2
        l6, s6 = diff(1, k2, k)
        l8, s8 = diff(0, k, k2)
        pp[(c, c2)] = [(l6, ((1, k2, n),), ((s6, 1, n), (s6, 1, n2))),
                       (("x", k2, k), ((1, k, n2), (1, k2, n)), ((1, 0, n), (-1, 1, n2))),
                       (l8, ((1, k, n2),), ((s8, 0, n), (s8, 0, n2)))]
        ext[c][0].append((1, k2, n))
        ext[c][1].append((-1, k, n2))
        ext[c2][0].append((1, k, n2))
        ext[c2][1].append((-1, k2, n))
    dp = {}
    for (k, n), t in diags.items():
        e0, e1 = ext[(k, n)]
        dp[(k, n)] = [(("p", 1 - t, k), ((1, k, n),) + tuple(e0), ((1, 1 - t, n), (1, t, n))),
                      (("x", k, k), ((1, k, n),) + tuple(e1), ((1 - 2 * t, t, n),))]
    return pp, dp


def _lhs_value(key, a):
    if key[0] == "d":
        return a(key[1], key[2]) - a(key[1], key[3])
    if key[0] == "x":
        return a(0, key[1]) - a(1, key[2])
    return a(key[1], key[2])


def _hk_double(n, cell0, cell1, shift=0):
    diags = {cell0(j): 0 for j in range(n)}
    diags.update({cell1(j): 1 for j in range(n)})
    pp, dp = _hk_plan(diags, [(cell0(j), cell1(l)) for j in range(n) for l in range(n) if j != l])
    order = []
    for j in range(n):
        for c in [(j, l) for l in range(n)] + [(l, (j + shift) % n) for l in range(n)]:
            if c[0] != c[1] and c not in order:
                order.append(c)
    rounds = []
    for j, l in order:
        rnd = list(pp[(cell0(j), cell1(l))])
        d = (l - j) % n
        if n == 5:
            rnd.append(dp[cell0(j)][d - 1] if d <= 2 else dp[cell1(l)][d - 3])
        else:
            rnd += [dp[cell0(j)][d - 1], dp[cell1(l)][d - 1]]
        rounds.append(rnd)
    return rounds


def _hk_double2():
    diags = {(j, j): 0 for j in range(5)}
    diags.update({(j, 5 + j): 1 for j in range(5)})
    pp, dp = _hk_plan(diags, [((j, j), (l, 5 + l)) for j in range(5) for l in range(5) if j != l])
    rounds = []
    for j in range(5):
        for l in range(j + 1, 5):
            own, kind = (j, l - j - 1) if l - j <= 2 else (l, j + 5 - l - 1)
            rounds.append(pp[((j, j), (l, 5 + l))] + pp[((l, l), (j, 5 + j))]
                          + [dp[(own, own)][kind], dp[(own, 5 + own)][kind]])
    return rounds


def _hk_single(c0, c1):
    pp, dp = _hk_plan({c0: 0, c1: 1}, [(c0, c1)])
    return pp[(c0, c1)] + dp[c0] + dp[c1]


UP_KEYS = ([("d", i, k2, k) for i in range(2) for k2 in range(5) for k in range(k2)]
           + [("x", k2, k) for k2 in range(5) for k in range(5) if k != k2]
           + [("x", k, k) for k in range(5)] + [("p", i, k) for i in range(2) for k in range(5)])


class _Hk:
    def __init__(self, r, mm, lhs, b, cache, fly, rows=128):
        self.r, self.mm, self.lhs, self.b, self.cache, self.fly = r, mm, lhs, b, cache, fly
        self.slot, self.rows = 0, rows

    def rhs(self, terms_list):
        out = []
        for terms in terms_list:
            if len(terms) == 1:
                out.append(self.b(*terms[0][1:]))
                continue
            ref = self.cache.at[self.slot]
            self.slot += 1
            if not self.fly:
                out.append(ref[...])
                continue
            s = self.b(*terms[0][1:]).astype(f32)
            for sg, k, n in terms[1:]:
                v = self.b(k, n).astype(f32)
                s = s + v if sg > 0 else s - v
            h = s.shape[0] // 2
            ref[0:h] = s[:h].astype(bf16)
            ref[h:2 * h] = s[h:].astype(bf16)
            out.append(s)
        return (out[0] if len(out) == 1 else jnp.concatenate(out, axis=0)).astype(bf16)

    def run(self, rounds, done):
        left = {}
        for rnd in rounds:
            for o in {(i, n) for _, _, outs in rnd for _, i, n in outs}:
                left[o] = left.get(o, 0) + 1
        acc = {}
        rows = self.rows
        part = self.r.part.at[:, 0:rows]
        for rnd in rounds:
            con, bykey = {}, {}
            for idx, p in enumerate(rnd):
                bykey.setdefault(p[0] if rows == 64 else idx, []).append(p)
            grps = sorted(bykey.values(), key=lambda g: -len(g))
            lv = [self.lhs(g[0][0]) for g in grps] if rows == 64 else None
            for gi, g in enumerate(grps):
                y = self.mm(lv[gi] if lv else self.lhs(g[0][0]), self.rhs([p[1] for p in g]))
                for t, p in enumerate(g):
                    for s, i, n in p[2]:
                        con.setdefault((i, n), []).append((s, y[rows * t:rows * (t + 1)]))
                yield len(g) * rows / 128
            for o, lst in con.items():
                lst.sort(key=lambda t: -t[0])
                s0, v = lst[0]
                for s, y in lst[1:]:
                    v = v + y if s == s0 else v - y
                if o in acc:
                    sa, _, sl = acc[o]
                    va = part[sl]
                    if sa == s0:
                        v = va + v
                    else:
                        v, s0 = (va - v, 1) if sa > 0 else (v - va, 1)
                else:
                    sl = self.r.pring[0]
                    self.r.pring[0] = (sl + 1) % NPART
                left[o] -= 1
                keep = left[o] == 0 and not (self.fly and rows == 128)
                if not keep:
                    part[sl] = v
                acc[o] = (s0, v if keep else None, sl)
            for n in sorted({n for _, n in con}):
                if left[(0, n)] == 0 and left[(1, n)] == 0:
                    h = [acc.pop((i, n)) for i in range(2)]
                    h = [(s, part[sl] if v is None else v) for s, v, sl in h]
                    done(n, jnp.concatenate([v if s > 0 else -v for s, v in h],
                                            axis=0 if rows == 128 else 1))


def _ffn(r, blk, solo):
    seen, cols = set(), {}

    def hl(key):
        ref = r.hs.at[UP_KEYS.index(key)]
        if key in seen:
            return ref[...]
        seen.add(key)
        v = _lhs_value(key, lambda i, k: r.hn[blk, 128 * i:128 * i + 128, 128 * k:128 * k + 128])
        ref[0:64] = v[:64].astype(bf16)
        ref[64:128] = v[64:].astype(bf16)
        return v.astype(bf16)

    def wu(k, n):
        return (r.w1, r.w3)[n[0]][128 * n[1]:128 * n[1] + 128, 128 * k:128 * k + 128]

    def act(c, g, u):
        hg = 0.5 * g
        a = (hg * jnp.tanh(hg) + hg) * u
        if c == 13:
            lane = jax.lax.broadcasted_iota(jnp.int32, a.shape, 1)
            a = jnp.where(lane < 64, a, 0.0)
        r.a[c] = a

    def updone(n, v):
        cols[n] = v
        if (1 - n[0], n[1]) in cols:
            act(n[1], cols.pop((0, n[1])), cols.pop((1, n[1])))

    wt = jnp.concatenate([r.w1[1664:1728], r.w3[1664:1728]], axis=0)
    g = _nt(r.hn[blk].astype(bf16), wt)
    yield 10
    act(13, g, pltpu.roll(g, 64, 1))
    up = _Hk(r, _nt, hl, wu, r.wup, solo)
    for c0, n in ((10, 3), (0, 5), (5, 5)):
        sh = SHIFT if n == 5 else 0
        plan = _hk_double(n, lambda j: (j, (0, c0 + j)), lambda j: (j, (1, c0 + (j - sh) % n)), sh)
        if n == 3:
            sing = [_hk_single((3, (0, c0 + j)), (4, (1, c0 + j))) for j in range(3)]
            plan = plan[:4] + sing[:1] + plan[4:] + sing[1:]
        yield from up.run(plan, updone)

    def al(key):
        return _lhs_value(key, lambda i, k: r.a[k, 128 * i:128 * i + 128]).astype(bf16)

    def wd(k, n):
        cs = slice(128 * n, 128 * n + 128)
        if k == 13:
            return jnp.concatenate([r.w2[1664:1728, cs], jnp.zeros((64, 128), bf16)], axis=0)
        return r.w2[128 * k:128 * k + 128, cs]

    def finish(n, y):
        cs = slice(128 * n, 128 * n + 128)
        r.o[blk, :, cs] = (r.h1[blk, :, cs] + y).astype(bf16)
        if solo:
            pltpu.make_async_copy(r.o.at[blk, :, cs], r.oh.at[blk, :, cs], r.osem).start()

    dn = _Hk(r, _nn, al, wd, r.wdn, solo)
    plan = [_hk_single((k, n), (k + 1, n + 1)) for n in (0, 2) for k in (10, 12)]
    plan += _hk_double(5, lambda j: (j, j), lambda j: (5 + j, j))
    yield from dn.run(plan, lambda n, y: finish(n, y) if n < 4 else cols.update(y4=y))
    a = jnp.concatenate([r.a[k] for k in range(10, 13)] + [r.a[13][:, :64]], axis=1).astype(bf16)
    y = cols["y4"] + _nn(a, r.w2[1280:1728, 512:640])
    yield 8
    finish(4, y)
    if not solo:
        pltpu.make_async_copy(r.o.at[blk], r.oh.at[blk], r.osem).start()


def _ln1(r, blk, rows=128):
    ps = list(_ln_pairs(lambda rs: r.x[blk, rs].astype(f32), rows))
    xf = jnp.concatenate([p[2] for p in ps] + [p[3] for p in ps], axis=0)
    r.xf[blk] = xf
    return xf, ps[-1][4][0:1]


class _Proj:
    def __init__(self, r, blk, qs, xf):
        self.r, self.blk, self.qs, self.xn = r, blk, qs, xf.astype(bf16)
        self.kt, self.qt = [], []

    def put(self, y):
        isq = len(self.qt) < 5
        tiles = self.qt if isq else self.kt
        tiles.append(y)
        for g in range(NW):
            if (80 * g + 79) // 128 == len(tiles) - 1:
                if isq:
                    self.r.q[self.qs, g] = _window(tiles, g) * QSCALE
                else:
                    self.r.k[self.blk, g] = _window(tiles, g).astype(bf16)

    def qk(self, p0, p1):
        y = _nn(self.xn, self.r.wqkv[:, 256 * p0:256 * p1])
        for t in range(2 * (p1 - p0)):
            self.put(y[:, 128 * t:128 * (t + 1)])

    def v(self, fly=False):
        r = self.r
        cols = {}

        def lhs(key):
            tile = lambda i, k: r.xf[self.blk, 128 * i:128 * i + 128, 128 * k:128 * k + 128]
            return _lhs_value(key, tile).astype(bf16)
        hk = _Hk(r, lambda a, b: _nt(b, a), lhs,
                 lambda k, n: r.wvt[64 * n:64 * n + 64, 128 * k:128 * k + 128], r.wvs, fly, 64)
        yield from hk.run(_hk_double2(), lambda n, y: cols.update({n: y}))
        vt = jnp.concatenate([cols[n] for n in range(10)], axis=0)
        sub8t = jax.lax.broadcasted_iota(jnp.int32, (8, T), 0)
        ones16 = jnp.ones((16, T), f32)
        ev, od = [], []
        for p in range(16):
            mid = vt[40 * p + 16:40 * p + 24]
            ev += [vt[40 * p:40 * p + 16], jnp.where(sub8t < 4, mid, 1.0), ones16]
            od += [ones16, jnp.where(sub8t < 4, 1.0, mid), vt[40 * p + 24:40 * p + 40]]
        for par, lst in enumerate((ev, od)):
            v = jnp.concatenate(lst, axis=0)
            for t in range(2):
                r.vt[self.blk, par, t] = v[:, 128 * t:128 * t + 128].astype(bf16)


class _Attn:
    def __init__(self, r, blk, first, qs, pin=None):
        self.r, self.blk, self.first, self.qs, self.pin = r, blk, first, qs, pin
        self.sc = {}
        self.units = [(self, b, g) for b in range(T // 128) for g in range(NW)]

    def scores(self, b, g):
        r, first = self.r, self.first
        cur, prev = self.blk, self.blk - 1
        lane32 = jax.lax.broadcasted_iota(jnp.int32, (32, 128), 1)
        row32 = jax.lax.broadcasted_iota(jnp.int32, (32, 128), 0)
        tri = row32 > (lane32 % 32)
        ns = []
        for j in range(4):
            q0 = 128 * b + 32 * j
            qsub = r.q[self.qs, g, q0:q0 + 32]
            parts = [None] * 4
            for h in range(4):
                lo = (80 * g + 20 * h) % 128
                hi = lo + 20
                if hi <= 128:
                    msk = (lane32 >= lo) & (lane32 < hi)
                else:
                    msk = (lane32 >= lo) | (lane32 < hi - 128)
                parts[(h + j) % 4] = jnp.where(msk, qsub, 0.0)
            wt = jnp.concatenate(parts, axis=0).astype(bf16)
            if first:
                s = _nt(r.k[cur, g, 0:q0 + 32], wt)
                lst = ([s[:q0]] if q0 else []) + [jnp.where(tri, NEG, s[q0:])]
                if j < 3:
                    lst.append(jnp.full((96 - 32 * j, 128), NEG, f32))
                ns.append(jnp.concatenate(lst, axis=0))
            else:
                def krows(r0, r1):
                    a0, a1 = q0 + r0, q0 + r1
                    if a0 == a1:
                        return []
                    if a1 <= T:
                        return [r.k[prev, g, a0:a1]]
                    if a0 >= T:
                        return [r.k[cur, g, a0 - T:a1 - T]]
                    return [r.k[prev, g, a0:T], r.k[cur, g, 0:a1 - T]]
                o = 32 * j
                kc = (krows(256 - o, 256) + krows(0, 16) + krows(256, 272) + krows(16, 32)
                      + krows(272, 288) + krows(32, 256 - o))
                s = _nt(jnp.concatenate(kc, axis=0), wt)
                top = jnp.concatenate([s[o:o + 16], s[o + 32:o + 48]], axis=0)
                bot = jnp.concatenate([s[o + 16:o + 32], s[o + 48:o + 64]], axis=0)
                mer = jnp.where(tri, top, bot)
                ns.append(jnp.concatenate(([s[:o]] if j else []) + [mer, s[o + 64:]], axis=0))
        lane = jax.lax.broadcasted_iota(jnp.int32, ns[0].shape, 1)
        odd = (lane % 64) >= 32
        aa = [jnp.where(odd, ns[(j + 1) % 4], ns[j]) for j in range(4)]
        out = []
        for h in range(4):
            j = (4 - h) % 4
            sm = jnp.where(lane >= 64, aa[(j + 2) % 4], aa[j])
            sl = r.ring[0]
            r.ring[0] = (sl + 1) % NRING
            n = sm.shape[0]
            r.s[sl, 0:n] = sm
            m = jnp.max(sm, axis=0, keepdims=True)
            if self.pin is not None and NW * b + g == PIN and h == 0:
                m = m + self.pin
            out.append((sl, n, m))
        self.sc[(b, g)] = out

    def softpv(self, b, g):
        r, first = self.r, self.first
        cur, prev = self.blk, self.blk - 1
        sub8 = jax.lax.broadcasted_iota(jnp.int32, (8, 128), 0)
        lane128 = jax.lax.broadcasted_iota(jnp.int32, (128, 128), 1)
        row128 = jax.lax.broadcasted_iota(jnp.int32, (128, 128), 0)
        ss = self.sc.pop((b, g))
        res = []
        for h in range(4):
            sl, n, m = ss[h]
            pm = jnp.exp2(r.s[sl, 0:n] - m)
            if not first:
                trih = row128 > ((lane128 + 128 - 32 * h) % 128)
                pm = jnp.concatenate([jnp.where(trih, pm[:128], 0.0), pm[128:],
                                      jnp.where(trih, 0.0, pm[:128])], axis=0)
            ph = pm.astype(bf16)
            r0 = 80 * g + 16 * h
            tl = [(cur, t) for t in range(b + 1)]
            if not first:
                tl = [(prev, t) for t in range(b, 2)] + tl
            vc = jnp.concatenate([r.vt[bk, h % 2, t, r0:r0 + 32] for bk, t in tl], axis=1)
            y = _nn(vc, ph)
            if h < 2:
                l, o = y[24:32], y[0:24]
            else:
                l, o = y[0:8], y[8:32]
            inv = 1.0 / l
            o = o * jnp.concatenate([inv, inv, inv], axis=0)
            if h:
                o = pltpu.roll(o, 128 - 32 * h, 1)
            res.append(o)
        rows = []
        for a, c in (res[0:2], res[2:4]):
            rows += [a[0:16], jnp.where(sub8 < 4, a[16:24], c[0:8]), c[8:24]]
        r.ot[self.qs, 80 * g:80 * g + 80, 128 * b:128 * b + 128] = jnp.concatenate(rows, axis=0)

    def oproj(self, fly, ln_rows):
        r, blk = self.r, self.blk
        cols = {}

        def lhs(key):
            tile = lambda i, k: r.ot[self.qs, 128 * k:128 * k + 128, 128 * i:128 * i + 128]
            return _lhs_value(key, tile).astype(bf16)

        def wt(k, n):
            r0 = 128 * (n % 5) + 64 * (n // 5)
            return r.wot[r0:r0 + 64, 128 * k:128 * k + 128]

        def done(n, v):
            cols[n] = v
            if n >= 5:
                cs = slice(128 * (n - 5), 128 * (n - 4))
                y = jnp.concatenate([cols[n - 5], v], axis=0).T
                r.h1[blk, :, cs] = r.x[blk, :, cs].astype(f32) + y
        hk = _Hk(r, lambda a, b: _nn(b, a), lhs, wt, r.wos, fly, 64)
        _Fill(hk.run(_hk_double2(), done)).advance()
        for ra, rb, ha, hb, _ in _ln_pairs(lambda rs: r.h1[blk, rs], ln_rows):
            r.hn[blk, ra] = ha
            r.hn[blk, rb] = hb


def _pipeline(units, lag, between):
    for i in range(len(units) + lag):
        if i < len(units):
            a, b, g = units[i]
            a.scores(b, g)
        between(i)
        if i >= lag:
            a, b, g = units[i - lag]
            a.softpv(b, g)


def _steady(r, blk):
    fill = _Fill(_ffn(r, blk - 1, False))
    p = _Proj(r, blk, 0, r.xf[blk])
    vf = _Fill(p.v())
    for t in range(5):
        p.qk(t, t + 1)
        vf.advance(8 * (t + 1))
    vf.advance()
    _, pin = _ln1(r, jnp.minimum(blk + 1, NB - 1), 8)
    at = _Attn(r, blk, False, 0, pin)
    _pipeline(at.units, LAG, lambda i: fill.advance(sum(SLOTS[:i + 1])))
    fill.advance(CMID)
    at.oproj(False, 32)
    fill.advance()


class _Refs:
    pass


def _kernel(x_h, wqkv_h, wo_h, w1_h, w3_h, w2_h, o_h,
            x_s, o_s, wqkv, wo, w1, w3, w2, wvt, wot, ot_s, wvs, wos, wup, wdn,
            k_s, vt_s, h1_s, hn_s, hs_s, a_s, p_s, xf_s, s_s, q_s, sems, osem):
    r = _Refs()
    r.x, r.o, r.wqkv, r.w1, r.w3, r.w2, r.wvt, r.wot = x_s, o_s, wqkv, w1, w3, w2, wvt, wot
    r.wvs, r.wos, r.wup, r.wdn, r.ot = wvs, wos, wup, wdn, ot_s
    r.k, r.vt, r.h1, r.hn, r.hs = k_s, vt_s, h1_s, hn_s, hs_s
    r.s, r.ring, r.q, r.xf = s_s, [0], q_s, xf_s
    r.oh, r.osem, r.a, r.part, r.pring = o_h, osem, a_s, p_s, [0]

    def xcopy(blk):
        return pltpu.make_async_copy(x_h.at[blk], x_s.at[blk], sems.at[8 + blk])

    def prologue():
        def wcol(c0, c1):
            return wqkv_h.at[:, c0:c1], wqkv.at[:, c0:c1]
        cx0, cx1, cx2 = xcopy(0), xcopy(1), xcopy(2)
        pairs = [wcol(0, 256), wcol(256, 768), wcol(768, 2 * D), wcol(2 * D, 3 * D),
                 (wo_h, wo), (w1_h, w1), (w3_h, w3), (w2_h, w2)]
        cps = [pltpu.make_async_copy(s, d, sems.at[i]) for i, (s, d) in enumerate(pairs)]
        for c in [cx0, cx1] + cps[:3] + [cx2] + cps[3:]:
            c.start()
        for blk in range(3, NB):
            xcopy(blk).start()
        ca, cb, cc, cv, cwo, cw1, cw3, cw2 = cps
        cx0.wait()
        p0 = _Proj(r, 0, 0, _ln1(r, 0)[0])
        cx1.wait()
        p1 = _Proj(r, 1, 1, _ln1(r, 1)[0])
        ca.wait()
        p0.qk(0, 1)
        p1.qk(0, 1)
        cb.wait()
        p0.qk(1, 3)
        p1.qk(1, 3)
        cc.wait()
        cx2.wait()
        p0.qk(3, 5)
        _ln1(r, 2, 16)
        p1.qk(3, 5)
        cv.wait()
        cwo.wait()
        wvt[...] = wqkv[:, 2 * D:3 * D].astype(f32).T.astype(bf16)
        wot[...] = wo[...].astype(f32).T.astype(bf16)
        a0, a1 = _Attn(r, 0, True, 0), _Attn(r, 1, False, 1)
        big = list(a1.units)
        small = sorted(a0.units, key=lambda u: (u[2], -u[1]))
        units, mid, k = big[:2], big[2:-3], 0
        for i, u in enumerate(mid):
            while k < len(small) and k * len(mid) < (i + 1) * len(small):
                units.append(small[k])
                k += 1
            units.append(u)
        units += big[-3:]

        def between(i):
            if i == LAGP:
                _Fill(p0.v(True)).advance()
                _Fill(p1.v()).advance()
            if i == len(units):
                a0.oproj(True, 64)
        _pipeline(units, LAGP, between)
        a1.oproj(False, 128)
        cw1.wait()
        cw3.wait()
        cw2.wait()

    def step(i, carry):
        pl.when(i == 0)(prologue)

        @pl.when((i > 1) & (i < NB))
        def _():
            pl.when(i < NB - 1)(lambda: xcopy(i + 1).wait())
            _steady(r, i)

        @pl.when((i == 1) | (i == NB))
        def _():
            _Fill(_ffn(r, i - 1, True)).advance()
        return carry
    jax.lax.fori_loop(0, NB + 1, step, 0)
    pltpu.make_async_copy(o_s, o_h, osem).wait()


@jax.jit
def pallas_sequential_preLN__sliding_block__glu_gated_swiglu__prompt_kernel(A_x, A_wqkv, A_wo, B_x, B_w1, B_w3, B_w2):
    del B_x
    x = A_x.reshape(NB, T, D)
    hbm = pl.BlockSpec(memory_space=pltpu.HBM)
    out = pl.pallas_call(
        _kernel,
        in_specs=[hbm] * 6,
        out_specs=hbm,
        out_shape=jax.ShapeDtypeStruct((NB, T, D), bf16),
        scratch_shapes=[
            pltpu.VMEM((NB, T, D), bf16), pltpu.VMEM((NB, T, D), bf16),
            pltpu.VMEM((D, 3 * D), bf16), pltpu.VMEM((D, D), bf16),
            pltpu.VMEM((F, D), bf16), pltpu.VMEM((F, D), bf16), pltpu.VMEM((F, D), bf16),
            pltpu.VMEM((D, D), bf16), pltpu.VMEM((D, D), bf16),
            pltpu.VMEM((2, D, T), f32),
            pltpu.VMEM((40, 64, 128), bf16), pltpu.VMEM((40, 64, 128), bf16),
            pltpu.VMEM((113, 128, 128), bf16), pltpu.VMEM((60, 128, 128), bf16),
            pltpu.VMEM((NB, NW, T, 128), bf16),
            pltpu.VMEM((NB, 2, 2, D, 128), bf16),
            pltpu.VMEM((NB, T, D), f32), pltpu.VMEM((NB, T, D), f32),
            pltpu.VMEM((55, 128, 128), bf16), pltpu.VMEM((14, T, 128), f32),
            pltpu.VMEM((NPART, 128, 128), f32), pltpu.VMEM((NB, T, D), f32),
            pltpu.VMEM((NRING, T, 128), f32), pltpu.VMEM((2, NW, T, 128), f32),
            pltpu.SemaphoreType.DMA((8 + NB,)), pltpu.SemaphoreType.DMA(()),
        ],
        compiler_params=pltpu.CompilerParams(
            vmem_limit_bytes=100 * 1024 * 1024,
            disable_bounds_checks=True, disable_semaphore_checks=True),
        name="fused_block",
    )(x, A_wqkv, A_wo, B_w1.T, B_w3.T, B_w2)
    return out.reshape(1, S, D)
```

```python
import math

import jax
import jax.numpy as jnp
import jax.experimental.pallas as pl
import jax.experimental.pallas.tpu as pltpu

S, D, DH, F = 2048, 640, 20, 1728
T = 256
NB = S // T
NW = 8
EPS = 1e-5
QSCALE = (DH ** -0.5) * math.log2(math.e)
NEG = -1e30
NRING = 16
NPART = 64
LAG = 1
LAGP = 2
SLOTS = [20, 20, 18] + [16] * 10 + [18, 16, 12, 12]
CMID = 288
SHIFT = 2
PIN = 12
f32 = jnp.float32
bf16 = jnp.bfloat16


def _ln_rows(x, dep):
    t = x[:, 0:128] if dep is None else x[:, 0:128] + dep
    for c in range(1, 5):
        t = t + x[:, 128 * c:128 * (c + 1)]
    m = jnp.sum(t, axis=-1, keepdims=True) * (1.0 / D)
    xc = x - m
    v = jnp.mean(xc * xc, axis=-1, keepdims=True)
    rs = jax.lax.rsqrt(v + EPS)
    return xc * rs, rs * 0.0


def _ln_pairs(load, rows):
    da = db = None
    for s in range(0, 128, rows):
        ra, rb = slice(s, s + rows), slice(128 + s, 128 + s + rows)
        a, da = _ln_rows(load(ra), da)
        b, db = _ln_rows(load(rb), db)
        yield ra, rb, a, b, da + db


def _window(tiles, g):
    t0, t1 = (80 * g) // 128, (80 * g + 79) // 128
    if t0 == t1:
        return tiles[t0]
    lane = jax.lax.broadcasted_iota(jnp.int32, tiles[t0].shape, 1)
    return jnp.where(lane >= (80 * g) % 128, tiles[t0], tiles[t1])


def _nn(a, b):
    return jnp.dot(a, b, preferred_element_type=f32)


def _nt(a, b):
    return jax.lax.dot_general(a, b, (((1,), (1,)), ((), ())), preferred_element_type=f32)


class _Fill:
    def __init__(self, gen):
        self.gen, self.done = gen, 0

    def advance(self, target=10 ** 9):
        while self.done < target:
            try:
                self.done += next(self.gen)
            except StopIteration:
                return


def _hk_plan(diags, pairs):
    def diff(i, k2, k):
        return (("d", i, k2, k), 1) if k2 > k else (("d", i, k, k2), -1)
    ext = {c: ([], []) for c in diags}
    pp = {}
    for c, c2 in pairs:
        (k, n), (k2, n2) = c, c2
        l6, s6 = diff(1, k2, k)
        l8, s8 = diff(0, k, k2)
        pp[(c, c2)] = [(l6, ((1, k2, n),), ((s6, 1, n), (s6, 1, n2))),
                       (("x", k2, k), ((1, k, n2), (1, k2, n)), ((1, 0, n), (-1, 1, n2))),
                       (l8, ((1, k, n2),), ((s8, 0, n), (s8, 0, n2)))]
        ext[c][0].append((1, k2, n))
        ext[c][1].append((-1, k, n2))
        ext[c2][0].append((1, k, n2))
        ext[c2][1].append((-1, k2, n))
    dp = {}
    for (k, n), t in diags.items():
        e0, e1 = ext[(k, n)]
        dp[(k, n)] = [(("p", 1 - t, k), ((1, k, n),) + tuple(e0), ((1, 1 - t, n), (1, t, n))),
                      (("x", k, k), ((1, k, n),) + tuple(e1), ((1 - 2 * t, t, n),))]
    return pp, dp


def _lhs_value(key, a):
    if key[0] == "d":
        return a(key[1], key[2]) - a(key[1], key[3])
    if key[0] == "x":
        return a(0, key[1]) - a(1, key[2])
    return a(key[1], key[2])


def _hk_double(cell0, cell1, shift=0):
    diags = {cell0(j): 0 for j in range(5)}
    diags.update({cell1(j): 1 for j in range(5)})
    pp, dp = _hk_plan(diags, [(cell0(j), cell1(l)) for j in range(5) for l in range(5) if j != l])
    order = []
    for j in range(5):
        for c in [(j, l) for l in range(5)] + [(l, (j + shift) % 5) for l in range(5)]:
            if c[0] != c[1] and c not in order:
                order.append(c)
    rounds = []
    for j, l in order:
        d = (l - j) % 5
        rounds.append(pp[(cell0(j), cell1(l))] + [dp[cell0(j)][d - 1] if d <= 2 else dp[cell1(l)][d - 3]])
    return rounds


def _hk_double2():
    diags = {(j, j): 0 for j in range(5)}
    diags.update({(j, 5 + j): 1 for j in range(5)})
    pp, dp = _hk_plan(diags, [((j, j), (l, 5 + l)) for j in range(5) for l in range(5) if j != l])
    rounds = []
    for j in range(5):
        for l in range(j + 1, 5):
            own, kind = (j, l - j - 1) if l - j <= 2 else (l, j + 5 - l - 1)
            rounds.append(pp[((j, j), (l, 5 + l))] + pp[((l, l), (j, 5 + j))]
                          + [dp[(own, own)][kind], dp[(own, 5 + own)][kind]])
    return rounds


def _hk_design(pairs, plain, km, nm, size):
    cell = lambda c: (km[c[0]], nm[c[1]])
    pairs = [(cell(c), cell(c2)) for c, c2 in pairs]
    diags = {c: t for p in pairs for t, c in enumerate(p)}
    pp, dp = _hk_plan(diags, pairs)
    rest = [p for c in diags for p in dp[c]]
    rest += [(("p", i, k), ((1, k, n),), ((1, i, n),)) for k, n in map(cell, plain) for i in range(2)]
    last = {n: max(j for j, p in enumerate(pairs) if n in (p[0][1], p[1][1])) for n in nm}
    rounds = []
    for j, p in enumerate(pairs):
        rnd = list(pp[p])
        cand = sorted((q for q in rest if q[2][0][2] in (p[0][1], p[1][1])), key=lambda q: last[q[2][0][2]])
        for q in cand:
            if len(rnd) < size or last[q[2][0][2]] == j:
                rnd.append(q)
                rest.remove(q)
        rounds.append(rnd)
    assert not rest
    return rounds


UP57 = ([((0, 3), (3, 5)), ((0, 3), (1, 6)), ((0, 3), (2, 4)), ((0, 3), (4, 0)), ((2, 5), (1, 6)),
         ((2, 5), (4, 0)), ((3, 2), (4, 0)), ((3, 2), (0, 1)), ((3, 2), (1, 6)), ((3, 2), (2, 4)),
         ((4, 1), (1, 6)), ((4, 1), (2, 4))], [(1, 0), (1, 4)])
DN45 = ([((0, 3), (1, 0)), ((0, 3), (2, 4)), ((0, 3), (3, 2)), ((1, 2), (2, 4)), ((3, 1), (1, 0)),
         ((3, 1), (2, 4))], [(0, 1), (2, 0)])
UP_KEYS = ([("d", i, k2, k) for i in range(2) for k2 in range(5) for k in range(k2)]
           + [("x", k2, k) for k2 in range(5) for k in range(5) if k != k2]
           + [("x", k, k) for k in range(5)] + [("p", i, k) for i in range(2) for k in range(5)])


class _Hk:
    def __init__(self, r, mm, lhs, b, cache, fly, rows=128):
        self.r, self.mm, self.lhs, self.b, self.cache, self.fly = r, mm, lhs, b, cache, fly
        self.slot, self.rows = 0, rows

    def rhs(self, terms_list):
        out = []
        for terms in terms_list:
            if len(terms) == 1:
                out.append(self.b(*terms[0][1:]))
                continue
            ref = self.cache.at[self.slot]
            self.slot += 1
            if not self.fly:
                out.append(ref[...])
                continue
            s = self.b(*terms[0][1:]).astype(f32)
            for sg, k, n in terms[1:]:
                v = self.b(k, n).astype(f32)
                s = s + v if sg > 0 else s - v
            h = s.shape[0] // 2
            ref[0:h] = s[:h].astype(bf16)
            ref[h:2 * h] = s[h:].astype(bf16)
            out.append(s)
        return (out[0] if len(out) == 1 else jnp.concatenate(out, axis=0)).astype(bf16)

    def run(self, rounds, done):
        left = {}
        for rnd in rounds:
            for o in {(i, n) for _, _, outs in rnd for _, i, n in outs}:
                left[o] = left.get(o, 0) + 1
        acc = {}
        rows = self.rows
        part = self.r.part.at[:, 0:rows]
        for rnd in rounds:
            con, bykey = {}, {}
            for idx, p in enumerate(rnd):
                bykey.setdefault(p[0] if rows == 64 else idx, []).append(p)
            grps = sorted(bykey.values(), key=lambda g: -len(g))
            lv = [self.lhs(g[0][0]) for g in grps] if rows == 64 else None
            for gi, g in enumerate(grps):
                y = self.mm(lv[gi] if lv else self.lhs(g[0][0]), self.rhs([p[1] for p in g]))
                for t, p in enumerate(g):
                    for s, i, n in p[2]:
                        con.setdefault((i, n), []).append((s, y[rows * t:rows * (t + 1)]))
                yield len(g) * rows / 128
            for o, lst in con.items():
                lst.sort(key=lambda t: -t[0])
                s0, v = lst[0]
                for s, y in lst[1:]:
                    v = v + y if s == s0 else v - y
                if o in acc:
                    sa, _, sl = acc[o]
                    va = part[sl]
                    if sa == s0:
                        v = va + v
                    else:
                        v, s0 = (va - v, 1) if sa > 0 else (v - va, 1)
                else:
                    sl = self.r.pring[0]
                    self.r.pring[0] = (sl + 1) % NPART
                left[o] -= 1
                keep = left[o] == 0 and not (self.fly and rows == 128)
                if not keep:
                    part[sl] = v
                acc[o] = (s0, v if keep else None, sl)
            for n in sorted({n for _, n in con}):
                if left[(0, n)] == 0 and left[(1, n)] == 0:
                    h = [acc.pop((i, n)) for i in range(2)]
                    h = [(s, part[sl] if v is None else v) for s, v, sl in h]
                    done(n, jnp.concatenate([v if s > 0 else -v for s, v in h],
                                            axis=0 if rows == 128 else 1))


def _ffn(r, blk, solo):
    seen, cols = set(), {}

    def hl(key):
        ref = r.hs.at[UP_KEYS.index(key)]
        if key in seen:
            return ref[...]
        seen.add(key)
        v = _lhs_value(key, lambda i, k: r.hn[blk, 128 * i:128 * i + 128, 128 * k:128 * k + 128])
        ref[0:64] = v[:64].astype(bf16)
        ref[64:128] = v[64:].astype(bf16)
        return v.astype(bf16)

    def wu(k, n):
        ks = slice(128 * k, 128 * k + 128)
        if n[1] == 13:
            return jnp.concatenate([r.w1[1664:1728, ks], r.w3[1664:1728, ks]], axis=0)
        return (r.w1, r.w3)[n[0]][128 * n[1]:128 * n[1] + 128, ks]

    def act(c, g, u):
        hg = 0.5 * g
        a = (hg * jnp.tanh(hg) + hg) * u
        if c == 13:
            lane = jax.lax.broadcasted_iota(jnp.int32, a.shape, 1)
            a = jnp.where(lane < 64, a, 0.0)
        r.a[c] = a

    def updone(n, v):
        cols[n] = v
        if n[1] == 13:
            act(13, v, pltpu.roll(v, 64, 1))
        elif (1 - n[0], n[1]) in cols:
            act(n[1], cols.pop((0, n[1])), cols.pop((1, n[1])))

    up = _Hk(r, _nt, hl, wu, r.wup, solo)
    nm = [(0, 11), (0, 12), (1, 11), (0, 10), (1, 12), (1, 10), (0, 13)]
    yield from up.run(_hk_design(*UP57, range(5), nm, 5), updone)
    for c0 in (0, 5):
        yield from up.run(_hk_double(lambda j: (j, (0, c0 + j)),
                                     lambda j: (j, (1, c0 + (j - SHIFT) % 5)), SHIFT), updone)

    def al(key):
        return _lhs_value(key, lambda i, k: r.a[k, 128 * i:128 * i + 128]).astype(bf16)

    def wd(k, n):
        cs = slice(128 * n, 128 * n + 128)
        if k == 13:
            return jnp.concatenate([r.w2[1664:1728, cs], jnp.zeros((64, 128), bf16)], axis=0)
        return r.w2[128 * k:128 * k + 128, cs]

    def finish(n, y):
        cs = slice(128 * n, 128 * n + 128)
        r.o[blk, :, cs] = (r.h1[blk, :, cs] + y).astype(bf16)
        if solo:
            pltpu.make_async_copy(r.o.at[blk, :, cs], r.oh.at[blk, :, cs], r.osem).start()

    dn = _Hk(r, _nn, al, wd, r.wdn, solo)
    plan = _hk_design(*DN45, range(10, 14), range(5), 6)
    plan += _hk_double(lambda j: (j, j), lambda j: (5 + j, j))
    yield from dn.run(plan, finish)
    if not solo:
        pltpu.make_async_copy(r.o.at[blk], r.oh.at[blk], r.osem).start()


def _ln1(r, blk, rows=128):
    ps = list(_ln_pairs(lambda rs: r.x[blk, rs].astype(f32), rows))
    xf = jnp.concatenate([p[2] for p in ps] + [p[3] for p in ps], axis=0)
    r.xf[blk] = xf
    return xf, ps[-1][4][0:1]


class _Proj:
    def __init__(self, r, blk, qs, xf):
        self.r, self.blk, self.qs, self.xn = r, blk, qs, xf.astype(bf16)
        self.kt, self.qt = [], []

    def put(self, y):
        isq = len(self.qt) < 5
        tiles = self.qt if isq else self.kt
        tiles.append(y)
        for g in range(NW):
            if (80 * g + 79) // 128 == len(tiles) - 1:
                if isq:
                    self.r.q[self.qs, g] = _window(tiles, g) * QSCALE
                else:
                    self.r.k[self.blk, g] = _window(tiles, g).astype(bf16)

    def qk(self, p0, p1):
        y = _nn(self.xn, self.r.wqkv[:, 256 * p0:256 * p1])
        for t in range(2 * (p1 - p0)):
            self.put(y[:, 128 * t:128 * (t + 1)])

    def v(self, fly=False):
        r = self.r
        cols = {}

        def lhs(key):
            tile = lambda i, k: r.xf[self.blk, 128 * i:128 * i + 128, 128 * k:128 * k + 128]
            return _lhs_value(key, tile).astype(bf16)
        hk = _Hk(r, lambda a, b: _nt(b, a), lhs,
                 lambda k, n: r.wvt[64 * n:64 * n + 64, 128 * k:128 * k + 128], r.wvs, fly, 64)
        yield from hk.run(_hk_double2(), lambda n, y: cols.update({n: y}))
        vt = jnp.concatenate([cols[n] for n in range(10)], axis=0)
        sub8t = jax.lax.broadcasted_iota(jnp.int32, (8, T), 0)
        ones16 = jnp.ones((16, T), f32)
        ev, od = [], []
        for p in range(16):
            mid = vt[40 * p + 16:40 * p + 24]
            ev += [vt[40 * p:40 * p + 16], jnp.where(sub8t < 4, mid, 1.0), ones16]
            od += [ones16, jnp.where(sub8t < 4, 1.0, mid), vt[40 * p + 24:40 * p + 40]]
        for par, lst in enumerate((ev, od)):
            v = jnp.concatenate(lst, axis=0)
            for t in range(2):
                r.vt[self.blk, par, t] = v[:, 128 * t:128 * t + 128].astype(bf16)


class _Attn:
    def __init__(self, r, blk, first, qs, pin=None):
        self.r, self.blk, self.first, self.qs, self.pin = r, blk, first, qs, pin
        self.sc = {}
        self.units = [(self, b, g) for b in range(T // 128) for g in range(NW)]

    def scores(self, b, g):
        r, first = self.r, self.first
        cur, prev = self.blk, self.blk - 1
        lane32 = jax.lax.broadcasted_iota(jnp.int32, (32, 128), 1)
        row32 = jax.lax.broadcasted_iota(jnp.int32, (32, 128), 0)
        tri = row32 > (lane32 % 32)
        ns = []
        for j in range(4):
            q0 = 128 * b + 32 * j
            qsub = r.q[self.qs, g, q0:q0 + 32]
            parts = [None] * 4
            for h in range(4):
                lo = (80 * g + 20 * h) % 128
                hi = lo + 20
                if hi <= 128:
                    msk = (lane32 >= lo) & (lane32 < hi)
                else:
                    msk = (lane32 >= lo) | (lane32 < hi - 128)
                parts[(h + j) % 4] = jnp.where(msk, qsub, 0.0)
            wt = jnp.concatenate(parts, axis=0).astype(bf16)
            if first:
                s = _nt(r.k[cur, g, 0:q0 + 32], wt)
                lst = ([s[:q0]] if q0 else []) + [jnp.where(tri, NEG, s[q0:])]
                if j < 3:
                    lst.append(jnp.full((96 - 32 * j, 128), NEG, f32))
                ns.append(jnp.concatenate(lst, axis=0))
            else:
                def krows(r0, r1):
                    a0, a1 = q0 + r0, q0 + r1
                    if a0 == a1:
                        return []
                    if a1 <= T:
                        return [r.k[prev, g, a0:a1]]
                    if a0 >= T:
                        return [r.k[cur, g, a0 - T:a1 - T]]
                    return [r.k[prev, g, a0:T], r.k[cur, g, 0:a1 - T]]
                o = 32 * j
                kc = (krows(256 - o, 256) + krows(0, 16) + krows(256, 272) + krows(16, 32)
                      + krows(272, 288) + krows(32, 256 - o))
                s = _nt(jnp.concatenate(kc, axis=0), wt)
                top = jnp.concatenate([s[o:o + 16], s[o + 32:o + 48]], axis=0)
                bot = jnp.concatenate([s[o + 16:o + 32], s[o + 48:o + 64]], axis=0)
                mer = jnp.where(tri, top, bot)
                ns.append(jnp.concatenate(([s[:o]] if j else []) + [mer, s[o + 64:]], axis=0))
        lane = jax.lax.broadcasted_iota(jnp.int32, ns[0].shape, 1)
        odd = (lane % 64) >= 32
        aa = [jnp.where(odd, ns[(j + 1) % 4], ns[j]) for j in range(4)]
        out = []
        for h in range(4):
            j = (4 - h) % 4
            sm = jnp.where(lane >= 64, aa[(j + 2) % 4], aa[j])
            sl = r.ring[0]
            r.ring[0] = (sl + 1) % NRING
            n = sm.shape[0]
            r.s[sl, 0:n] = sm
            m = jnp.max(sm, axis=0, keepdims=True)
            if self.pin is not None and NW * b + g == PIN and h == 0:
                m = m + self.pin
            out.append((sl, n, m))
        self.sc[(b, g)] = out

    def softpv(self, b, g):
        r, first = self.r, self.first
        cur, prev = self.blk, self.blk - 1
        sub8 = jax.lax.broadcasted_iota(jnp.int32, (8, 128), 0)
        lane128 = jax.lax.broadcasted_iota(jnp.int32, (128, 128), 1)
        row128 = jax.lax.broadcasted_iota(jnp.int32, (128, 128), 0)
        ss = self.sc.pop((b, g))
        res = []
        for h in range(4):
            sl, n, m = ss[h]
            pm = jnp.exp2(r.s[sl, 0:n] - m)
            if not first:
                trih = row128 > ((lane128 + 128 - 32 * h) % 128)
                pm = jnp.concatenate([jnp.where(trih, pm[:128], 0.0), pm[128:],
                                      jnp.where(trih, 0.0, pm[:128])], axis=0)
            ph = pm.astype(bf16)
            r0 = 80 * g + 16 * h
            tl = [(cur, t) for t in range(b + 1)]
            if not first:
                tl = [(prev, t) for t in range(b, 2)] + tl
            vc = jnp.concatenate([r.vt[bk, h % 2, t, r0:r0 + 32] for bk, t in tl], axis=1)
            y = _nn(vc, ph)
            if h < 2:
                l, o = y[24:32], y[0:24]
            else:
                l, o = y[0:8], y[8:32]
            inv = 1.0 / l
            o = o * jnp.concatenate([inv, inv, inv], axis=0)
            if h:
                o = pltpu.roll(o, 128 - 32 * h, 1)
            res.append(o)
        rows = []
        for a, c in (res[0:2], res[2:4]):
            rows += [a[0:16], jnp.where(sub8 < 4, a[16:24], c[0:8]), c[8:24]]
        r.ot[self.qs, 80 * g:80 * g + 80, 128 * b:128 * b + 128] = jnp.concatenate(rows, axis=0)

    def oproj(self, fly, ln_rows):
        r, blk = self.r, self.blk
        cols = {}

        def lhs(key):
            tile = lambda i, k: r.ot[self.qs, 128 * k:128 * k + 128, 128 * i:128 * i + 128]
            return _lhs_value(key, tile).astype(bf16)

        def wt(k, n):
            r0 = 128 * (n % 5) + 64 * (n // 5)
            return r.wot[r0:r0 + 64, 128 * k:128 * k + 128]

        def done(n, v):
            cols[n] = v
            if n >= 5:
                cs = slice(128 * (n - 5), 128 * (n - 4))
                y = jnp.concatenate([cols[n - 5], v], axis=0).T
                r.h1[blk, :, cs] = r.x[blk, :, cs].astype(f32) + y
        hk = _Hk(r, lambda a, b: _nn(b, a), lhs, wt, r.wos, fly, 64)
        _Fill(hk.run(_hk_double2(), done)).advance()
        for ra, rb, ha, hb, _ in _ln_pairs(lambda rs: r.h1[blk, rs], ln_rows):
            r.hn[blk, ra] = ha
            r.hn[blk, rb] = hb


def _pipeline(units, lag, between):
    for i in range(len(units) + lag):
        if i < len(units):
            a, b, g = units[i]
            a.scores(b, g)
        between(i)
        if i >= lag:
            a, b, g = units[i - lag]
            a.softpv(b, g)


def _steady(r, blk):
    fill = _Fill(_ffn(r, blk - 1, False))
    p = _Proj(r, blk, 0, r.xf[blk])
    vf = _Fill(p.v())
    for t in range(5):
        p.qk(t, t + 1)
        vf.advance(8 * (t + 1))
    vf.advance()
    _, pin = _ln1(r, jnp.minimum(blk + 1, NB - 1), 8)
    at = _Attn(r, blk, False, 0, pin)
    _pipeline(at.units, LAG, lambda i: fill.advance(sum(SLOTS[:i + 1])))
    fill.advance(CMID)
    at.oproj(False, 32)
    fill.advance()


class _Refs:
    pass


def _kernel(x_h, wqkv_h, wo_h, w1_h, w3_h, w2_h, o_h,
            x_s, o_s, wqkv, wo, w1, w3, w2, wvt, wot, ot_s, wvs, wos, wup, wdn,
            k_s, vt_s, h1_s, hn_s, hs_s, a_s, p_s, xf_s, s_s, q_s, sems, osem):
    r = _Refs()
    r.x, r.o, r.wqkv, r.w1, r.w3, r.w2, r.wvt, r.wot = x_s, o_s, wqkv, w1, w3, w2, wvt, wot
    r.wvs, r.wos, r.wup, r.wdn, r.ot = wvs, wos, wup, wdn, ot_s
    r.k, r.vt, r.h1, r.hn, r.hs = k_s, vt_s, h1_s, hn_s, hs_s
    r.s, r.ring, r.q, r.xf = s_s, [0], q_s, xf_s
    r.oh, r.osem, r.a, r.part, r.pring = o_h, osem, a_s, p_s, [0]

    def xcopy(blk):
        return pltpu.make_async_copy(x_h.at[blk], x_s.at[blk], sems.at[8 + blk])

    def prologue():
        def wcol(c0, c1):
            return wqkv_h.at[:, c0:c1], wqkv.at[:, c0:c1]
        cx0, cx1, cx2 = xcopy(0), xcopy(1), xcopy(2)
        pairs = [wcol(0, 256), wcol(256, 768), wcol(768, 2 * D), wcol(2 * D, 3 * D),
                 (wo_h, wo), (w1_h, w1), (w3_h, w3), (w2_h, w2)]
        cps = [pltpu.make_async_copy(s, d, sems.at[i]) for i, (s, d) in enumerate(pairs)]
        for c in [cx0, cx1] + cps[:3] + [cx2] + cps[3:]:
            c.start()
        for blk in range(3, NB):
            xcopy(blk).start()
        ca, cb, cc, cv, cwo, cw1, cw3, cw2 = cps
        cx0.wait()
        p0 = _Proj(r, 0, 0, _ln1(r, 0)[0])
        cx1.wait()
        p1 = _Proj(r, 1, 1, _ln1(r, 1)[0])
        ca.wait()
        p0.qk(0, 1)
        p1.qk(0, 1)
        cb.wait()
        p0.qk(1, 3)
        p1.qk(1, 3)
        cc.wait()
        cx2.wait()
        p0.qk(3, 5)
        _ln1(r, 2, 16)
        p1.qk(3, 5)
        cv.wait()
        cwo.wait()
        wvt[...] = wqkv[:, 2 * D:3 * D].astype(f32).T.astype(bf16)
        wot[...] = wo[...].astype(f32).T.astype(bf16)
        a0, a1 = _Attn(r, 0, True, 0), _Attn(r, 1, False, 1)
        big = list(a1.units)
        small = sorted(a0.units, key=lambda u: (u[2], -u[1]))
        units, mid, k = big[:2], big[2:-3], 0
        for i, u in enumerate(mid):
            while k < len(small) and k * len(mid) < (i + 1) * len(small):
                units.append(small[k])
                k += 1
            units.append(u)
        units += big[-3:]

        def between(i):
            if i == LAGP:
                _Fill(p0.v(True)).advance()
                _Fill(p1.v()).advance()
            if i == len(units):
                a0.oproj(True, 64)
        _pipeline(units, LAGP, between)
        a1.oproj(False, 128)
        cw1.wait()
        cw3.wait()
        cw2.wait()

    def step(i, carry):
        pl.when(i == 0)(prologue)

        @pl.when((i > 1) & (i < NB))
        def _():
            pl.when(i < NB - 1)(lambda: xcopy(i + 1).wait())
            _steady(r, i)

        @pl.when((i == 1) | (i == NB))
        def _():
            _Fill(_ffn(r, i - 1, True)).advance()
        return carry
    jax.lax.fori_loop(0, NB + 1, step, 0)
    pltpu.make_async_copy(o_s, o_h, osem).wait()


@jax.jit
def pallas_sequential_preLN__sliding_block__glu_gated_swiglu__prompt_kernel(A_x, A_wqkv, A_wo, B_x, B_w1, B_w3, B_w2):
    del B_x
    x = A_x.reshape(NB, T, D)
    hbm = pl.BlockSpec(memory_space=pltpu.HBM)
    out = pl.pallas_call(
        _kernel,
        in_specs=[hbm] * 6,
        out_specs=hbm,
        out_shape=jax.ShapeDtypeStruct((NB, T, D), bf16),
        scratch_shapes=[
            pltpu.VMEM((NB, T, D), bf16), pltpu.VMEM((NB, T, D), bf16),
            pltpu.VMEM((D, 3 * D), bf16), pltpu.VMEM((D, D), bf16),
            pltpu.VMEM((F, D), bf16), pltpu.VMEM((F, D), bf16), pltpu.VMEM((F, D), bf16),
            pltpu.VMEM((D, D), bf16), pltpu.VMEM((D, D), bf16),
            pltpu.VMEM((2, D, T), f32),
            pltpu.VMEM((40, 64, 128), bf16), pltpu.VMEM((40, 64, 128), bf16),
            pltpu.VMEM((110, 128, 128), bf16), pltpu.VMEM((58, 128, 128), bf16),
            pltpu.VMEM((NB, NW, T, 128), bf16),
            pltpu.VMEM((NB, 2, 2, D, 128), bf16),
            pltpu.VMEM((NB, T, D), f32), pltpu.VMEM((NB, T, D), f32),
            pltpu.VMEM((55, 128, 128), bf16), pltpu.VMEM((14, T, 128), f32),
            pltpu.VMEM((NPART, 128, 128), f32), pltpu.VMEM((NB, T, D), f32),
            pltpu.VMEM((NRING, T, 128), f32), pltpu.VMEM((2, NW, T, 128), f32),
            pltpu.SemaphoreType.DMA((8 + NB,)), pltpu.SemaphoreType.DMA(()),
        ],
        compiler_params=pltpu.CompilerParams(
            vmem_limit_bytes=100 * 1024 * 1024,
            disable_bounds_checks=True, disable_semaphore_checks=True),
        name="fused_block",
    )(x, A_wqkv, A_wo, B_w1.T, B_w3.T, B_w2)
    return out.reshape(1, S, D)
```
